```python
import os as _os
_os.environ.setdefault("JAX_PLATFORMS", "cpu")
import jax
import jax.numpy as jnp

def _softmax(x, axis=-1):
    return jax.nn.softmax(x, axis=axis)
def _gelu(x):
    return jax.nn.gelu(x, approximate=True)
def _silu(x):
    return jax.nn.silu(x)
def _sigmoid(x):
    return jax.nn.sigmoid(x)
def _layernorm(x, axis=-1, eps=1e-5):
    m = jnp.mean(x, axis=axis, keepdims=True)
    v = jnp.var(x, axis=axis, keepdims=True)
    return (x - m) / jnp.sqrt(v + eps)
def _scatter_add(tgt, idx, src, axis=0):
    return tgt.at[idx].add(src)
def _segment_sum(src, seg, n):
    return jax.ops.segment_sum(src, seg, n)
class _Rng:
    def __init__(self, key):
        self._k = key
    def _next(self):
        self._k, sub = jax.random.split(self._k)
        return sub
    def normal(self, shape):
        return jax.random.normal(self._next(), shape, dtype=jnp.bfloat16)
    def randint(self, lo, hi, shape):
        return jax.random.randint(self._next(), shape, lo, hi, dtype=jnp.int32)
    def uniform(self, shape, lo=0.0, hi=1.0):
        return jax.random.uniform(self._next(), shape, jnp.bfloat16, lo, hi)
    def permutation(self, n):
        return jax.random.permutation(self._next(), n)


kernel_name = 'standalone__gqa_block_cached__near_ridge'

def setup_inputs():
    _rng = _Rng(jax.random.key(int.from_bytes(__import__("os").urandom(4), "little")))
    _w = (lambda a: (lambda t: t.astype(jnp.bfloat16) if jnp.issubdtype(t.dtype, jnp.floating) else t)(jnp.asarray(a)))
    B, Sq, D = 16, 128, 576
    Hq, Hkv, Sk, Dh = 32, 16, 1024, 128
    assert Hq % Hkv == 0, (Hq, Hkv)
    return {
        "x": _w((lambda *s: _rng.normal(s) * 0.8)(B, Sq, D)),
        "k_cache": _w((lambda *s: _rng.normal(s) * 0.8)(B, Hkv, Sk, Dh)),
        "v_cache": _w((lambda *s: _rng.normal(s) * 0.05)(B, Hkv, Sk, Dh)),
        "wq": _w((lambda *s: _rng.normal(s) * 0.8)(D, Hq * Dh) * (D ** -0.5)),
        "wo": _w((lambda *s: _rng.normal(s) * 0.05)(Hq * Dh, D) * ((Hq * Dh) ** -0.5)),
    }

def reference(x, k_cache, v_cache, wq, wo):
    B, Sq, D = x.shape
    Hq, Dh = 32, 128
    Hkv = k_cache.shape[1]
    rep = Hq // Hkv
    q = (lambda x, *d: x.transpose(*d))((x @ wq).reshape(B, Sq, Hq, Dh), 0, 2, 1, 3)
    k = jnp.repeat(k_cache, rep, axis=1)
    v = jnp.repeat(v_cache, rep, axis=1)
    scores = jnp.einsum("bhqd,bhkd->bhqk", q, k) * (Dh ** -0.5)
    p = _softmax(scores, axis=-1)
    o = jnp.einsum("bhqk,bhkd->bhqd", p, v)
    return (lambda x, *d: x.transpose(*d))(o, 0, 2, 1, 3).reshape(B, Sq, Hq * Dh) @ wo
```

```python
import functools

import jax
import jax.numpy as jnp
import jax.experimental.pallas as pl
import jax.experimental.pallas.tpu as pltpu

LOG2E = 1.4426950408889634
G = 2
NSLOW = 3
WIN = 2
JK = 1
NEXT = {0: ((0,), (1,)), 1: ((0, 1, 2), (3, 4, 5))}
NT = (((1,), (1,)), ((), ()))
f32, bf16 = jnp.float32, jnp.bfloat16


def _kernel(xt_hbm, k_hbm, v_hbm, wq_hbm, wot_hbm, out_ref,
            x_scr, q_scr, o_scr, acc_scr, x1_scr, q1_scr, o0_scr, acc0_scr, k_buf, v_buf, wq_v, wot_v,
            xt_buf, kv_sem, w_sem, kvw_sem, x_sem, *, rep, dh):
    b = pl.program_id(0)
    nb = pl.num_programs(0) - 1
    hkv = k_hbm.shape[1]
    sq = xt_hbm.shape[2]
    scale = (dh ** -0.5) * LOG2E
    W = rep * dh
    NG = hkv // G
    slot = b % 2

    def kv_copies(bb, sl, j):
        hs = pl.ds(j * G, G)
        return (pltpu.make_async_copy(k_hbm.at[bb, hs], k_buf.at[sl, hs], kv_sem.at[sl, 0, j]),
                pltpu.make_async_copy(v_hbm.at[bb, hs], v_buf.at[sl, hs], kv_sem.at[sl, 1, j]))

    def w_copy(src, dst, i, j):
        c = pl.ds(pl.multiple_of(j * G * W, G * W), G * W)
        return pltpu.make_async_copy(src.at[:, c], dst.at[j], w_sem.at[i, j])

    def x_copy(bb):
        sl = (bb + 1) % 2
        return pltpu.make_async_copy(xt_hbm.at[bb], xt_buf.at[sl], x_sem.at[sl])

    def wq_copy(j):
        return w_copy(wq_hbm, wq_v, 0, j)

    def wo_copy(j):
        return w_copy(wot_hbm, wot_v, 1, j)

    def kv_whole(bb, sl):
        return (pltpu.make_async_copy(k_hbm.at[bb], k_buf.at[sl], kvw_sem.at[sl, 0]),
                pltpu.make_async_copy(v_hbm.at[bb], v_buf.at[sl], kvw_sem.at[sl, 1]))

    def chunk_copies(step, j):
        cs = [(c, None) for c in kv_copies(step, step % 2, j)]
        if step == 0:
            cs.append((wq_copy(jnp.minimum(j + 1, NG - 1)), j + 1 < NG))
        if step == 1:
            cs.append((wo_copy(j), None))
        return cs

    def for_chunk(step, j, fn):
        for c, cond in chunk_copies(step, j):
            if cond is None or cond is True:
                fn(c)
            elif cond is not False:
                pl.when(cond)(functools.partial(fn, c))

    def start(c):
        c.start()

    def wait(c):
        c.wait()

    def advance(step, j):
        for_chunk(step, j, wait)
        static = isinstance(j, int)
        if step == 0 or step == 1:
            win = WIN
            if static:
                if j + win < NG:
                    for_chunk(step, j + win, start)
            else:
                pl.when(j + win < NG)(lambda: for_chunk(step, jnp.minimum(j + win, NG - 1), start))
            nxt = NEXT[step]
            if static and j == NG - 1:
                for jn in nxt[1]:
                    for_chunk(step + 1, jn, start)
            if not static:
                @pl.when(j == NG - 2)
                def _():
                    for jn in nxt[0]:
                        for_chunk(step + 1, jn, start)
        else:
            if static and j == 0:
                for jn in range(len(NEXT[1][0]) + len(NEXT[1][1]), NG):
                    for_chunk(step, jn, start)
            if not static:
                @pl.when(j == JK)
                def _():
                    for c in kv_whole(step + 1, (step + 1) % 2):
                        c.start()

    @pl.when(b == 0)
    def _():
        x_copy(0).start()
        wq_copy(0).start()
        x_copy(1).start()

    @pl.when(jnp.logical_and(b >= NSLOW, b + 1 < nb))
    def _():
        for c in kv_whole(b + 1, 1 - slot):
            c.start()

    @pl.when(jnp.logical_and(b >= 1, b + 1 < nb))
    def _():
        x_copy(b + 1).wait()

    @pl.when(jnp.logical_and(b >= 1, b + 2 < nb))
    def _():
        x_copy(b + 2).start()

    def qproj(j, x_src, q_dst):
        q = jnp.dot(x_src[...], wq_v[j], preferred_element_type=f32)
        for t in range(G * rep):
            h, r = j * G + t // rep, t % rep
            q_dst[h, r * sq:(r + 1) * sq, :] = (q[:, t * dh:(t + 1) * dh] * scale).astype(bf16)

    def qk(h, sl, q_src):
        return jax.lax.dot_general(q_src[h], k_buf[sl, h], NT, preferred_element_type=f32)

    def pv(j, i, s, sl, o_dst):
        h = j * G + i
        m = jnp.max(s, axis=-1, keepdims=True)
        p = jnp.exp2(s - m)
        l = jnp.sum(p, axis=-1, keepdims=True)
        o = jnp.dot(p.astype(bf16), v_buf[sl, h], preferred_element_type=f32)
        r_l = pl.reciprocal(l, approx=True)
        r_l = r_l * (2.0 - l * r_l)
        for r in range(rep):
            rows = slice(r * sq, (r + 1) * sq)
            o_dst[j, :, i * W + r * dh:i * W + (r + 1) * dh] = (o[rows] * r_l[rows]).astype(bf16)

    def oproj(j, o_src, acc, first=False, last=False):
        r = jax.lax.dot_general(wot_v[j], o_src[j], NT, preferred_element_type=f32)
        if not isinstance(first, bool):
            acc[...] = r + jnp.where(first, 0.0, acc[...])
        elif first:
            acc[...] = r
        elif last:
            out_ref[...] = (acc[...] + r).astype(out_ref.dtype)
        else:
            acc[...] += r

    def filler_a(step, j, first, last):
        if step == 1:
            oproj(j, o0_scr, acc0_scr, first=first, last=last)
        elif not last:
            qproj(j + 1, x_scr, q_scr)

    def filler_b(step, j, first, last):
        if step == 0:
            qproj(j, x1_scr, q1_scr)
        elif first:
            if step != 1:
                oproj(NG - 1, o_scr, acc_scr, last=True)
        else:
            oproj(j - 1, o_scr, acc_scr, first=(j == 1))

    def stage(step, j, first, last, adv=True):
        sl = slot if step is None else step % 2
        if step is not None and adv:
            advance(step, j)
        for i, filler in enumerate((filler_a, filler_b)):
            s = qk(j * G + i, sl, q1_scr if step == 1 else q_scr)
            filler(step, j, first, last)
            pv(j, i, s, sl, o0_scr if step == 0 else o_scr)
        if last and step != 0:
            x_scr[...] = xt_buf[slot].T
            qproj(0, x_scr, q_scr)

    def loop(step, lo, hi):
        def f(j, c):
            stage(step, j, False, False)
            return c
        jax.lax.fori_loop(lo, hi, f, 0)

    def body(step):
        if step == 0:
            x_copy(0).wait()
            x_copy(1).wait()
            for j in range(WIN):
                for_chunk(0, j, start)
            x_scr[...] = xt_buf[1].T
            x1_scr[...] = xt_buf[0].T
            x_copy(2).start()
            wq_copy(0).wait()
            qproj(0, x_scr, q_scr)
            loop(0, 0, NG - 1)
            stage(0, NG - 1, False, True)
        elif step is not None:
            stage(step, 0, True, False)
            if step + 1 == NSLOW:
                def pair(t, c):
                    j = 1 + 2 * t
                    advance(step, j)
                    advance(step, j + 1)
                    stage(step, j, False, False, adv=False)
                    stage(step, j + 1, False, False, adv=False)
                    return c
                jax.lax.fori_loop(0, (NG - 2) // 2, pair, 0)
            else:
                loop(step, 1, NG - 1)
            stage(step, NG - 1, False, True)
        else:
            for c in kv_whole(b, slot):
                c.wait()
            for j in range(NG):
                stage(None, j, j == 0, j + 1 == NG)

    for step in range(NSLOW):
        pl.when(b == step)(functools.partial(body, step))
    pl.when(jnp.logical_and(b >= NSLOW, b < nb))(lambda: body(None))
    pl.when(b == nb)(lambda: oproj(NG - 1, o_scr, acc_scr, last=True))


@jax.jit
def pallas_standalone__gqa_block_cached__near_ridge_kernel(x, k_cache, v_cache, wq, wo):
    B, Sq, D = x.shape
    _, Hkv, Sk, Dh = k_cache.shape
    Hq = wq.shape[1] // Dh
    rep = Hq // Hkv
    assert Hkv == 8 * G and B > NSLOW, "the DMA schedule is written for 8 stages per batch"
    NG, CW = Hkv // G, G * rep * Dh
    V = pltpu.VMEM
    any_spec = pl.BlockSpec(memory_space=pl.ANY)
    xt = x.transpose(0, 2, 1)
    out_t = pl.pallas_call(
        functools.partial(_kernel, rep=rep, dh=Dh),
        grid=(B + 1,),
        in_specs=[
            any_spec, any_spec, any_spec, any_spec, any_spec],
        out_specs=pl.BlockSpec((None, D, Sq), lambda b: (jnp.maximum(b - 1, 0), 0, 0)),
        out_shape=jax.ShapeDtypeStruct((B, D, Sq), x.dtype),
        scratch_shapes=[
            V((Sq, D), bf16), V((Hkv, rep * Sq, Dh), bf16),
            V((NG, Sq, CW), bf16), V((D, Sq), f32),
            V((Sq, D), bf16), V((Hkv, rep * Sq, Dh), bf16), V((NG, Sq, CW), bf16), V((D, Sq), f32),
            V((2, Hkv, Sk, Dh), bf16), V((2, Hkv, Sk, Dh), bf16), V((NG, D, CW), bf16), V((NG, D, CW), bf16),
            V((2, D, Sq), bf16),
            pltpu.SemaphoreType.DMA((2, 2, Hkv // G)), pltpu.SemaphoreType.DMA((2, Hkv // G)),
            pltpu.SemaphoreType.DMA((2, 2)), pltpu.SemaphoreType.DMA((2,)),
        ],
        compiler_params=pltpu.CompilerParams(
            dimension_semantics=("arbitrary",),
            vmem_limit_bytes=100 * 1024 * 1024,
        ),
    )(xt, k_cache, v_cache, wq, wo.T)
    return out_t.transpose(0, 2, 1)
```
